```python
import os as _os
_os.environ.setdefault("JAX_PLATFORMS", "cpu")
import jax
import jax.numpy as jnp

def _softmax(x, axis=-1):
    return jax.nn.softmax(x, axis=axis)
def _gelu(x):
    return jax.nn.gelu(x, approximate=True)
def _silu(x):
    return jax.nn.silu(x)
def _sigmoid(x):
    return jax.nn.sigmoid(x)
def _layernorm(x, axis=-1, eps=1e-5):
    m = jnp.mean(x, axis=axis, keepdims=True)
    v = jnp.var(x, axis=axis, keepdims=True)
    return (x - m) / jnp.sqrt(v + eps)
def _scatter_add(tgt, idx, src, axis=0):
    return tgt.at[idx].add(src)
def _segment_sum(src, seg, n):
    return jax.ops.segment_sum(src, seg, n)
class _Rng:
    def __init__(self, key):
        self._k = key
    def _next(self):
        self._k, sub = jax.random.split(self._k)
        return sub
    def normal(self, shape):
        return jax.random.normal(self._next(), shape, dtype=jnp.bfloat16)
    def randint(self, lo, hi, shape):
        return jax.random.randint(self._next(), shape, lo, hi, dtype=jnp.int32)
    def uniform(self, shape, lo=0.0, hi=1.0):
        return jax.random.uniform(self._next(), shape, jnp.bfloat16, lo, hi)
    def permutation(self, n):
        return jax.random.permutation(self._next(), n)


kernel_name = 'gated_mix__linear_attn_block__mixer_token_mlp__prompt'

def setup_inputs():
    _rng = _Rng(jax.random.key(int.from_bytes(__import__("os").urandom(4), "little")))
    _w = (lambda a: (lambda t: t.astype(jnp.bfloat16) if jnp.issubdtype(t.dtype, jnp.floating) else t)(jnp.asarray(a)))
    def _A_setup():
        B, S, D = 1, 2048, 512
        return {
            "x": _w((lambda *s: _rng.normal(s) * 0.05)(B, S, D)),
            "wqkv": _w((lambda *s: _rng.normal(s) * 0.8)(D, 3 * D)),
            "wo": _w((lambda *s: _rng.normal(s) * 0.05)(D, D)),
        }
    _A_in = _A_setup()

    def _B_setup():
        B, S, D, F = 1, 2048, 512, 1792
        return {
            "x": _w((lambda *s: _rng.normal(s) * 0.05)(B, S, D)),
            "w1": _w((lambda *s: _rng.normal(s) * 0.1)(S, F) * (S ** -0.5)),
            "b1": _w((lambda *s: _rng.normal(s) * 0.1)(F) * 0.02),
            "w2": _w((lambda *s: _rng.normal(s) * 0.1)(F, S) * (F ** -0.5)),
            "b2": _w((lambda *s: _rng.normal(s) * 0.1)(S) * 0.02),
        }
    _B_in = _B_setup()

    return {
        "A_x": _A_in["x"],
        "A_wqkv": _A_in["wqkv"],
        "A_wo": _A_in["wo"],
        "B_x": _B_in["x"],
        "B_w1": _B_in["w1"],
        "B_b1": _B_in["b1"],
        "B_w2": _B_in["w2"],
        "B_b2": _B_in["b2"],
        "gate_w": _w((lambda *s: _rng.normal(s) * 0.05)(512) * 16.0),
    }

def reference(A_x, A_wqkv, A_wo, B_x, B_w1, B_b1, B_w2, B_b2, gate_w):
    def _A_ref(x, wqkv, wo):
        B, S, D = x.shape
        H = 32; Dh = D // H
        qkv = (lambda x, *d: x.transpose(*d))((x @ wqkv).reshape(B, S, 3, H, Dh), 2, 0, 3, 1, 4)
        q, k, v = qkv[0], qkv[1], qkv[2]
        phi = lambda t: jnp.where(t > 0, t + 1, jnp.exp(t)) + 1e-6
        pq, pk = phi(q), phi(k)
        kv = jnp.einsum("bhsd,bhse->bhde", pk, v)
        z = jnp.einsum("bhsd->bhd", pk)
        num = jnp.einsum("bhqd,bhde->bhqe", pq, kv)
        den = jnp.einsum("bhqd,bhd->bhq", pq, z)[..., None] + 1e-6
        o = num / den
        return (lambda x, *d: x.transpose(*d))(o, 0, 2, 1, 3).reshape(B, S, D) @ wo

    def _B_ref(x, w1, b1, w2, b2):
        B, S, D = x.shape
        h = _layernorm(x, axis=-1)
        u = jnp.einsum("bsd,sf->bdf", h, w1) + b1
        u = _gelu(u)
        y = jnp.einsum("bdf,fs->bds", u, w2) + b2
        return (lambda x, *d: x.transpose(*d))(y, 0, 2, 1)

    x = A_x
    g = _sigmoid((x * gate_w).sum(-1, keepdims=True))
    a = _A_ref(x, A_wqkv, A_wo)
    b = _B_ref(x, B_w1, B_b1, B_w2, B_b2)
    return g * a + (1 - g) * b
```

```python
import functools

import jax
import jax.numpy as jnp
from jax import lax
import jax.experimental.pallas as pl
import jax.experimental.pallas.tpu as pltpu

F32 = jnp.float32
BF16 = jnp.bfloat16


def _phi(t):
    return jnp.where(t > 0, t + 1.0, jnp.exp(t)) + 1e-6


def _gelu_tanh(x):
    c = 0.7978845608028654
    return 0.5 * x * (1.0 + jnp.tanh(c * (x + 0.044715 * (x * x * x))))


def _kernel(x_hbm, wqkv_hbm, wo_hbm, w1_hbm, w2_hbm, b1_ref, b2_ref, gw_ref,
            out_hbm,
            x_v, wqkv_v, wo_v, w1_v, w2_v, wkT_v, pq_v, u_acc, kv_acc, z_acc,
            gu_v, M_v, Z_v, ostage,
            sem_x, sem_w1, sem_w2, sem_misc, sem_out,
            *, S, D, F, H, TS):
    NT = S // TS
    Dh = D // H
    NB = D // 128
    FC = F // NT

    def x_copy(i):
        return pltpu.make_async_copy(
            x_hbm.at[pl.ds(i * TS, TS), :], x_v.at[pl.ds(i * TS, TS), :], sem_x.at[i])

    def w1_copy(i):
        return pltpu.make_async_copy(
            w1_hbm.at[pl.ds(i * TS, TS), :], w1_v.at[pl.ds(i * TS, TS), :], sem_w1.at[i])

    def w2_copy(i):
        return pltpu.make_async_copy(
            w2_hbm.at[pl.ds(i * FC, FC), :], w2_v.at[pl.ds(i * FC, FC), :], sem_w2.at[i])

    def wqkv_copy():
        return pltpu.make_async_copy(wqkv_hbm, wqkv_v, sem_misc.at[0])

    def wo_copy():
        return pltpu.make_async_copy(wo_hbm, wo_v, sem_misc.at[1])

    def out_copy(i, slot):
        return pltpu.make_async_copy(
            ostage.at[slot], out_hbm.at[pl.ds(i * TS, TS), :], sem_out.at[slot])

    x_copy(0).start()
    w1_copy(0).start()
    wqkv_copy().start()
    x_copy(1).start()
    w1_copy(1).start()
    wo_copy().start()

    u_acc[...] = jnp.zeros(u_acc.shape, F32)
    kv_acc[...] = jnp.zeros(kv_acc.shape, F32)
    z_acc[...] = jnp.zeros(z_acc.shape, F32)

    wqkv_copy().wait()
    wkT_v[...] = wqkv_v[:, D:2 * D].astype(F32).T.astype(BF16)

    def p1_body(i, carry):
        s0 = pl.multiple_of(i * TS, TS)

        @pl.when(i + 2 < NT)
        def _():
            x_copy(i + 2).start()
            w1_copy(i + 2).start()

        w2_copy(i).start()

        x_copy(i).wait()
        x_t = x_v[pl.ds(s0, TS), :]
        xT = x_t.astype(F32).T
        mean = jnp.mean(xT, axis=0, keepdims=True)
        xc = xT - mean
        var = jnp.mean(xc * xc, axis=0, keepdims=True)
        hT = (xc * lax.rsqrt(var + 1e-5)).astype(BF16)

        w1_copy(i).wait()
        u_acc[...] += jnp.dot(hT, w1_v[pl.ds(s0, TS), :], preferred_element_type=F32)

        q = jnp.dot(x_t, wqkv_v[:, 0:D], preferred_element_type=F32)
        v = jnp.dot(x_t, wqkv_v[:, 2 * D:3 * D], preferred_element_type=F32)
        kT = jnp.dot(wkT_v[...], xT.astype(BF16), preferred_element_type=F32)
        pq_v[pl.ds(s0, TS), :] = _phi(q).astype(BF16)
        pkT = _phi(kT)
        zs = pkT[:, 0:128]
        for c in range(1, TS // 128):
            zs = zs + pkT[:, c * 128:(c + 1) * 128]
        z_acc[...] += zs
        pkT_b = pkT.astype(BF16)
        v_b = v.astype(BF16)
        for j in range(NB):
            kv_acc[j] += jnp.dot(pkT_b[j * 128:(j + 1) * 128, :],
                                 v_b[:, j * 128:(j + 1) * 128],
                                 preferred_element_type=F32)
        return carry

    lax.fori_loop(0, NT, p1_body, 0)

    gu_v[...] = _gelu_tanh(u_acc[...] + b1_ref[...].astype(F32)).astype(BF16)

    r_id = lax.broadcasted_iota(jnp.int32, (128, 128), 0) // Dh
    c_id = lax.broadcasted_iota(jnp.int32, (128, 128), 1) // Dh
    blk = r_id == c_id
    z_col = jnp.sum(z_acc[...], axis=1, keepdims=True)
    wo_copy().wait()
    for j in range(NB):
        kvj = jnp.where(blk, kv_acc[j], 0.0).astype(BF16)
        M_v[j * 128:(j + 1) * 128, :] = jnp.dot(
            kvj, wo_v[j * 128:(j + 1) * 128, :], preferred_element_type=F32).astype(BF16)
        Z_v[j] = jnp.where(blk, z_col[j * 128:(j + 1) * 128, :], 0.0).astype(BF16)

    for i in range(NT):
        w2_copy(i).wait()

    gw = gw_ref[...].astype(F32)

    def p2_body(i, carry):
        s0 = pl.multiple_of(i * TS, TS)
        slot = lax.rem(i, 2)

        pq_t = pq_v[pl.ds(s0, TS), :]
        den = jnp.concatenate(
            [jnp.dot(pq_t[:, j * 128:(j + 1) * 128], Z_v[j], preferred_element_type=F32)
             for j in range(NB)], axis=1) + 1e-6
        pqs = (pq_t.astype(F32) / den).astype(BF16)
        a = jnp.dot(pqs, M_v[...], preferred_element_type=F32)

        y = jnp.dot(gu_v[...], w2_v[:, pl.ds(s0, TS)], preferred_element_type=F32)
        y = y + b2_ref[:, pl.ds(s0, TS)].astype(F32)
        yT = y.T

        x_t = x_v[pl.ds(s0, TS), :].astype(F32)
        g = jax.nn.sigmoid(jnp.sum(x_t * gw, axis=1, keepdims=True))
        o = g * a + (1.0 - g) * yT

        @pl.when(i >= 2)
        def _():
            out_copy(i - 2, slot).wait()

        ostage[slot] = o.astype(BF16)
        out_copy(i, slot).start()
        return carry

    lax.fori_loop(0, NT, p2_body, 0)
    out_copy(NT - 2, (NT - 2) % 2).wait()
    out_copy(NT - 1, (NT - 1) % 2).wait()


@jax.jit
def pallas_gated_mix__linear_attn_block__mixer_token_mlp__prompt_kernel(
    A_x: jax.Array,
    A_wqkv: jax.Array,
    A_wo: jax.Array,
    B_x: jax.Array,
    B_w1: jax.Array,
    B_b1: jax.Array,
    B_w2: jax.Array,
    B_b2: jax.Array,
    gate_w: jax.Array,
):
    del B_x
    B, S, D = A_x.shape
    F = B_w1.shape[1]
    H = 32
    TS = 256
    NT = S // TS
    assert B == 1 and S % TS == 0 and F % NT == 0 and D % 128 == 0

    x = A_x.reshape(S, D)
    b1 = B_b1.reshape(1, F)
    b2 = B_b2.reshape(1, S)
    gw = gate_w.reshape(1, D)

    kernel = functools.partial(_kernel, S=S, D=D, F=F, H=H, TS=TS)
    any_spec = pl.BlockSpec(memory_space=pl.ANY)
    out = pl.pallas_call(
        kernel,
        out_shape=jax.ShapeDtypeStruct((S, D), A_x.dtype),
        in_specs=[any_spec, any_spec, any_spec, any_spec, any_spec,
                  pl.BlockSpec(memory_space=pltpu.VMEM),
                  pl.BlockSpec(memory_space=pltpu.VMEM),
                  pl.BlockSpec(memory_space=pltpu.VMEM)],
        out_specs=any_spec,
        scratch_shapes=[
            pltpu.VMEM((S, D), BF16),
            pltpu.VMEM((D, 3 * D), BF16),
            pltpu.VMEM((D, D), BF16),
            pltpu.VMEM((S, F), BF16),
            pltpu.VMEM((F, S), BF16),
            pltpu.VMEM((D, D), BF16),
            pltpu.VMEM((S, D), BF16),
            pltpu.VMEM((D, F), F32),
            pltpu.VMEM((D // 128, 128, 128), F32),
            pltpu.VMEM((D, 128), F32),
            pltpu.VMEM((D, F), BF16),
            pltpu.VMEM((D, D), BF16),
            pltpu.VMEM((D // 128, 128, 128), BF16),
            pltpu.VMEM((2, TS, D), BF16),
            pltpu.SemaphoreType.DMA((NT,)),
            pltpu.SemaphoreType.DMA((NT,)),
            pltpu.SemaphoreType.DMA((NT,)),
            pltpu.SemaphoreType.DMA((2,)),
            pltpu.SemaphoreType.DMA((2,)),
        ],
        compiler_params=pltpu.CompilerParams(
            vmem_limit_bytes=100 * 1024 * 1024,
        ),
    )(x, A_wqkv, A_wo, B_w1, B_w2, b1, b2, gw)
    return out.reshape(B, S, D)
```

```python
import functools

import jax
import jax.numpy as jnp
from jax import lax
import jax.experimental.pallas as pl
import jax.experimental.pallas.tpu as pltpu

F32 = jnp.float32
BF16 = jnp.bfloat16


def _phi(t):
    return jnp.where(t > 0, t + 1.0, jnp.exp(t)) + 1e-6


def _gelu_tanh(x):
    c = 0.7978845608028654
    inner = x * (c + (c * 0.044715) * (x * x))
    hx = 0.5 * x
    return hx + hx * jnp.tanh(inner)


def _kernel(x_hbm, wqkv_hbm, wo_hbm, w1_hbm, w2_hbm, b1_ref, b2_ref, gw_ref,
            out_hbm,
            x_v, wqkv_v, wo_v, w1_v, w2_v, wkT_v, pq_v, u_acc, kv_acc, z_acc,
            gu_v, M_v, Z_v, ostage, hA, hB, xA, xB, aA, aB, yA, yB, pA, pB,
            sem_x, sem_w1, sem_w2, sem_misc, sem_out,
            *, S, D, F, H, TS):
    NT = S // TS
    Dh = D // H
    NB = D // 128
    FC = F // NT
    PR = 64

    def x_copy(i):
        return pltpu.make_async_copy(
            x_hbm.at[pl.ds(i * TS, TS), :], x_v.at[pl.ds(i * TS, TS), :], sem_x.at[i])

    def w1_copy(i):
        return pltpu.make_async_copy(
            w1_hbm.at[pl.ds(i * TS, TS), :], w1_v.at[pl.ds(i * TS, TS), :], sem_w1.at[i])

    def w2_copy(i):
        return pltpu.make_async_copy(
            w2_hbm.at[pl.ds(i * FC, FC), :], w2_v.at[pl.ds(i * FC, FC), :], sem_w2.at[i])

    def wqkv_copy():
        return pltpu.make_async_copy(wqkv_hbm, wqkv_v, sem_misc.at[0])

    def wo_copy():
        return pltpu.make_async_copy(wo_hbm, wo_v, sem_misc.at[1])

    def out_copy(i):
        return pltpu.make_async_copy(
            ostage.at[pl.ds(i * TS, TS), :], out_hbm.at[pl.ds(i * TS, TS), :], sem_out.at[i])

    x_copy(0).start()
    w1_copy(0).start()

    def p1_prep(i, h_buf, xt_buf):
        s0 = pl.multiple_of(i * TS, TS)
        x_t = x_v[pl.ds(s0, TS), :]
        xT = x_t.astype(F32).T
        mean = jnp.mean(xT, axis=0, keepdims=True)
        xc = xT - mean
        var = jnp.mean(xc * xc, axis=0, keepdims=True)
        h_buf[...] = (xc * lax.rsqrt(var + 1e-5)).astype(BF16)
        xt_buf[...] = xT.astype(BF16)

    def p1_u(i, h_buf, first=False):
        s0 = pl.multiple_of(i * TS, TS)
        u = jnp.dot(h_buf[...], w1_v[pl.ds(s0, TS), :], preferred_element_type=F32)
        if first:
            u_acc[...] = u
        else:
            u_acc[...] += u

    def p1_main(i, h_buf, xt_buf, first=False):
        s0 = pl.multiple_of(i * TS, TS)
        x_t = x_v[pl.ds(s0, TS), :]
        kT = jnp.dot(wkT_v[...], xt_buf[...], preferred_element_type=F32)
        q = jnp.dot(x_t, wqkv_v[:, 0:D], preferred_element_type=F32)
        v = jnp.dot(x_t, wqkv_v[:, 2 * D:3 * D], preferred_element_type=F32)
        pkT = _phi(kT)
        zs = pkT[:, 0:128]
        for c in range(1, TS // 128):
            zs = zs + pkT[:, c * 128:(c + 1) * 128]
        if first:
            z_acc[...] = zs
        else:
            z_acc[...] += zs
        pkT_b = pkT.astype(BF16)
        v_b = v.astype(BF16)
        pq_v[pl.ds(s0, TS), :] = _phi(q).astype(BF16)
        if not first:
            p1_u(i, h_buf)
        for j in range(NB):
            kvj = jnp.dot(pkT_b[j * 128:(j + 1) * 128, :],
                          v_b[:, j * 128:(j + 1) * 128],
                          preferred_element_type=F32)
            if first:
                kv_acc[j] = kvj
            else:
                kv_acc[j] += kvj

    x_copy(0).wait()
    wqkv_copy().start()
    x_copy(1).start()
    p1_prep(0, hA, xA)
    w1_copy(0).wait()
    p1_u(0, hA, first=True)
    wqkv_copy().wait()
    w1_copy(1).start()
    x_copy(2).start()
    w1_copy(2).start()
    x_copy(1).wait()
    wkT_v[...] = wqkv_v[:, D:2 * D].astype(F32).T.astype(BF16)
    p1_main(0, hA, xA, first=True)
    p1_prep(1, hB, xB)

    def p1_body(k, carry):
        i = 2 * k + 1
        x_copy(i + 2).start()
        w1_copy(i + 2).start()
        x_copy(i + 1).wait()
        w1_copy(i).wait()
        p1_main(i, hB, xB)
        p1_prep(i + 1, hA, xA)

        @pl.when(i + 3 < NT)
        def _():
            x_copy(i + 3).start()
            w1_copy(i + 3).start()

        w2_copy(2 * k).start()
        w2_copy(2 * k + 1).start()
        x_copy(i + 2).wait()
        w1_copy(i + 1).wait()
        p1_main(i + 1, hA, xA)
        p1_prep(i + 2, hB, xB)
        return carry

    lax.fori_loop(0, NT // 2 - 1, p1_body, 0)
    wo_copy().start()
    w2_copy(NT - 2).start()
    w2_copy(NT - 1).start()
    w1_copy(NT - 1).wait()
    p1_main(NT - 1, hB, xB)

    RC = 16
    b1_row = b1_ref[...].astype(F32).reshape(1, F)
    for r in range(0, D, RC):
        gu_v[r:r + RC, :] = _gelu_tanh(
            u_acc[r:r + RC, :] + b1_row).astype(BF16)

    r_id = lax.broadcasted_iota(jnp.int32, (128, 128), 0) // Dh
    c_id = lax.broadcasted_iota(jnp.int32, (128, 128), 1) // Dh
    blk = r_id == c_id
    z_col = jnp.sum(z_acc[...], axis=1, keepdims=True)
    wo_copy().wait()
    for j in range(NB):
        kvj = jnp.where(blk, kv_acc[j], 0.0).astype(BF16)
        M_v[j * 128:(j + 1) * 128, :] = jnp.dot(
            kvj, wo_v[j * 128:(j + 1) * 128, :], preferred_element_type=F32).astype(BF16)
        Z_v[j] = jnp.where(blk, z_col[j * 128:(j + 1) * 128, :], 0.0).astype(BF16)

    for i in range(NT):
        w2_copy(i).wait()

    gw = gw_ref[...].astype(F32).reshape(1, D)

    def p2_pre(i, p_buf):
        s0 = pl.multiple_of(i * TS, TS)
        for r in range(0, TS, PR):
            pq_t = pq_v[pl.ds(s0 + r, PR), :]
            den = jnp.concatenate(
                [jnp.dot(pq_t[:, j * 128:(j + 1) * 128], Z_v[j], preferred_element_type=F32)
                 for j in range(NB)], axis=1) + 1e-6
            rcp = pl.reciprocal(den, approx=True)
            rcp = rcp * (2.0 - den * rcp)
            p_buf[r:r + PR, :] = (pq_t.astype(F32) * rcp).astype(BF16)

    def p2_main(i, p_buf, a_buf, y_buf):
        s0 = pl.multiple_of(i * TS, TS)
        y_buf[...] = jnp.dot(gu_v[...], w2_v[:, pl.ds(s0, TS)],
                             preferred_element_type=F32)
        a_buf[...] = jnp.dot(p_buf[...], M_v[...], preferred_element_type=F32)

    def p2_post(i, a_buf, y_buf):
        s0 = pl.multiple_of(i * TS, TS)
        y = y_buf[...] + b2_ref[pl.ds(s0, TS)].astype(F32).reshape(1, TS)
        yT = y.T
        x_t = x_v[pl.ds(s0, TS), :].astype(F32)
        g = jax.nn.sigmoid(jnp.sum(x_t * gw, axis=1, keepdims=True))
        o = g * a_buf[...] + (1.0 - g) * yT
        ostage[pl.ds(s0, TS), :] = o.astype(BF16)
        out_copy(i).start()

    p2_pre(0, pA)
    p2_main(0, pA, aA, yA)
    p2_pre(1, pB)

    def p2_body(k, carry):
        i = 2 * k
        p2_pre(i + 2, pA)
        p2_main(i + 1, pB, aB, yB)
        p2_post(i, aA, yA)
        p2_pre(i + 3, pB)
        p2_main(i + 2, pA, aA, yA)
        p2_post(i + 1, aB, yB)
        return carry

    lax.fori_loop(0, NT // 2 - 1, p2_body, 0)
    p2_main(NT - 1, pB, aB, yB)
    p2_post(NT - 2, aA, yA)
    p2_post(NT - 1, aB, yB)
    for i in range(NT):
        out_copy(i).wait()


@jax.jit
def pallas_gated_mix__linear_attn_block__mixer_token_mlp__prompt_kernel(
    A_x: jax.Array,
    A_wqkv: jax.Array,
    A_wo: jax.Array,
    B_x: jax.Array,
    B_w1: jax.Array,
    B_b1: jax.Array,
    B_w2: jax.Array,
    B_b2: jax.Array,
    gate_w: jax.Array,
):
    del B_x
    B, S, D = A_x.shape
    F = B_w1.shape[1]
    H = 32
    TS = 256
    NT = S // TS
    assert B == 1 and S % TS == 0 and F % NT == 0 and D % 128 == 0 and NT % 2 == 0

    x = A_x.reshape(S, D)
    b1 = B_b1
    b2 = B_b2
    gw = gate_w

    kernel = functools.partial(_kernel, S=S, D=D, F=F, H=H, TS=TS)
    any_spec = pl.BlockSpec(memory_space=pl.ANY)
    out = pl.pallas_call(
        kernel,
        out_shape=jax.ShapeDtypeStruct((S, D), A_x.dtype),
        in_specs=[any_spec, any_spec, any_spec, any_spec, any_spec,
                  pl.BlockSpec(memory_space=pltpu.VMEM),
                  pl.BlockSpec(memory_space=pltpu.VMEM),
                  pl.BlockSpec(memory_space=pltpu.VMEM)],
        out_specs=any_spec,
        scratch_shapes=[
            pltpu.VMEM((S, D), BF16),
            pltpu.VMEM((D, 3 * D), BF16),
            pltpu.VMEM((D, D), BF16),
            pltpu.VMEM((S, F), BF16),
            pltpu.VMEM((F, S), BF16),
            pltpu.VMEM((D, D), BF16),
            pltpu.VMEM((S, D), BF16),
            pltpu.VMEM((D, F), F32),
            pltpu.VMEM((D // 128, 128, 128), F32),
            pltpu.VMEM((D, 128), F32),
            pltpu.VMEM((D, F), BF16),
            pltpu.VMEM((D, D), BF16),
            pltpu.VMEM((D // 128, 128, 128), BF16),
            pltpu.VMEM((S, D), BF16),
            pltpu.VMEM((D, TS), BF16),
            pltpu.VMEM((D, TS), BF16),
            pltpu.VMEM((D, TS), BF16),
            pltpu.VMEM((D, TS), BF16),
            pltpu.VMEM((TS, D), F32),
            pltpu.VMEM((TS, D), F32),
            pltpu.VMEM((D, TS), F32),
            pltpu.VMEM((D, TS), F32),
            pltpu.VMEM((TS, D), BF16),
            pltpu.VMEM((TS, D), BF16),
            pltpu.SemaphoreType.DMA((NT,)),
            pltpu.SemaphoreType.DMA((NT,)),
            pltpu.SemaphoreType.DMA((NT,)),
            pltpu.SemaphoreType.DMA((2,)),
            pltpu.SemaphoreType.DMA((NT,)),
        ],
        compiler_params=pltpu.CompilerParams(
            vmem_limit_bytes=100 * 1024 * 1024,
        ),
    )(x, A_wqkv, A_wo, B_w1, B_w2, b1, b2, gw)
    return out.reshape(B, S, D)
```
